```python
import jax
import jax.numpy as jnp

def _softmax(x, axis=-1):
    return jax.nn.softmax(x, axis=axis)
def _gelu(x):
    return jax.nn.gelu(x, approximate=True)
def _silu(x):
    return jax.nn.silu(x)
def _sigmoid(x):
    return jax.nn.sigmoid(x)
def _layernorm(x, axis=-1, eps=1e-5):
    m = jnp.mean(x, axis=axis, keepdims=True)
    v = jnp.var(x, axis=axis, keepdims=True)
    return (x - m) / jnp.sqrt(v + eps)
def _scatter_add(tgt, idx, src, axis=0):
    return tgt.at[idx].add(src)
def _segment_sum(src, seg, n):
    return jax.ops.segment_sum(src, seg, n)
class _Rng:
    def __init__(self, key):
        self._k = key
    def _next(self):
        self._k, sub = jax.random.split(self._k)
        return sub
    def normal(self, shape):
        return jax.random.normal(self._next(), shape, dtype=jnp.bfloat16)
    def randint(self, lo, hi, shape):
        return jax.random.randint(self._next(), shape, lo, hi, dtype=jnp.int32)
    def uniform(self, shape, lo=0.0, hi=1.0):
        return jax.random.uniform(self._next(), shape, jnp.bfloat16, lo, hi)
    def permutation(self, n):
        return jax.random.permutation(self._next(), n)


kernel_name = 'parallel_sum__sliding_block_cached__moe_arch_mod__decode'

def setup_inputs():
    _rng = _Rng(jax.random.key(int.from_bytes(__import__("os").urandom(4), "little")))
    _w = (lambda a: (lambda t: t.astype(jnp.bfloat16) if jnp.issubdtype(t.dtype, jnp.floating) else t)(jnp.asarray(a)))
    def _A_setup():
        B, Sq, D = 1, 1, 512
        Hq, Hkv, Sk, Dh = 32, 8, 65536, 128
        assert Hq % Hkv == 0, (Hq, Hkv)
        return {
            "x": _w((lambda *s: _rng.normal(s) * 0.05)(B, Sq, D)),
            "k_cache": _w((lambda *s: _rng.normal(s) * 0.05)(B, Hkv, Sk, Dh)),
            "v_cache": _w((lambda *s: _rng.normal(s) * 0.05)(B, Hkv, Sk, Dh)),
            "wq": _w((lambda *s: _rng.normal(s) * 0.05)(D, Hq * Dh) * (D ** -0.5)),
            "wo": _w((lambda *s: _rng.normal(s) * 0.05)(Hq * Dh, D) * ((Hq * Dh) ** -0.5)),
        }
    _A_in = _A_setup()

    def _B_setup():
        B, S, D, F, C = 1, 1, 512, 1792, 1
        return {
            "x": _w((lambda *s: _rng.normal(s) * 0.05)(B, S, D)),
            "w_r": _w((lambda *s: _rng.normal(s) * 0.05)(D)),
            "w_gate": _w((lambda *s: _rng.normal(s) * 0.05)(D, F)),
            "w_up": _w((lambda *s: _rng.normal(s) * 0.05)(D, F)),
            "w_down": _w((lambda *s: _rng.normal(s) * 0.05)(F, D)),
        }
    _B_in = _B_setup()

    return {
        "A_x": _A_in["x"],
        "A_k_cache": _A_in["k_cache"],
        "A_v_cache": _A_in["v_cache"],
        "A_wq": _A_in["wq"],
        "A_wo": _A_in["wo"],
        "B_x": _B_in["x"],
        "B_w_r": _B_in["w_r"],
        "B_w_gate": _B_in["w_gate"],
        "B_w_up": _B_in["w_up"],
        "B_w_down": _B_in["w_down"],
    }

def reference(A_x, A_k_cache, A_v_cache, A_wq, A_wo, B_x, B_w_r, B_w_gate, B_w_up, B_w_down):
    def _A_ref(x, k_cache, v_cache, wq, wo):
        B, Sq, D = x.shape
        Hq, Dh = 32, 128
        Hkv, Sk = k_cache.shape[1], k_cache.shape[2]
        W = min(4096, max(256, Sk // 4))
        rep = Hq // Hkv
        q = (lambda x, *d: x.transpose(*d))((x @ wq).reshape(B, Sq, Hq, Dh), 0, 2, 1, 3)
        k = jnp.repeat(k_cache[:, :, Sk - W:, :], rep, axis=1)
        v = jnp.repeat(v_cache[:, :, Sk - W:, :], rep, axis=1)
        scores = jnp.einsum("bhqd,bhkd->bhqk", q, k) * (Dh ** -0.5)
        p = _softmax(scores, axis=-1)
        o = jnp.einsum("bhqk,bhkd->bhqd", p, v)
        return (lambda x, *d: x.transpose(*d))(o, 0, 2, 1, 3).reshape(B, Sq, Hq * Dh) @ wo

    def _B_ref(x, w_r, w_gate, w_up, w_down):
        B, S, D = x.shape
        C = 1
        r = x @ w_r
        idx = jnp.argsort(-r, axis=-1)[:, :C]
        idx_e = jnp.repeat(idx.reshape(B, C, 1), D, axis=2)
        x_sel = jnp.take_along_axis(x, idx_e, axis=1)
        g = _silu(x_sel @ w_gate)
        u = x_sel @ w_up
        y = (g * u) @ w_down
        r_sel = _sigmoid(jnp.take_along_axis(r, idx, axis=1))
        y = y * r_sel.reshape(B, C, 1)
        b_off = (jnp.arange(B) * S).reshape(B, 1)
        flat_idx = (idx + b_off).reshape(B * C)
        zero = (x * 0.0).reshape(B * S, D)
        upd = _scatter_add(zero, flat_idx, y.reshape(B * C, D), axis=0)
        return x + upd.reshape(B, S, D)

    x = A_x
    xn = _layernorm(x, axis=-1)
    return x + _A_ref(xn, A_k_cache, A_v_cache, A_wq, A_wo) + _B_ref(xn, B_w_r, B_w_gate, B_w_up, B_w_down)
```

```python
import jax
import jax.numpy as jnp
import jax.experimental.pallas as pl
import jax.experimental.pallas.tpu as pltpu

HQ, DH = 32, 128
LN_EPS = 1e-5
N_SEM = 4
WQ_CHUNKS = 4
_NN = (((1,), (0,)), ((), ()))
_NT = (((1,), (1,)), ((), ()))


def _dot(a, b, dims=_NN):
    return jax.lax.dot_general(a, b, dims, preferred_element_type=jnp.float32)


def _down_splits(f):
    vpu = (128, 128, 64, 64) if f >= 512 and f % 128 == 0 else ()
    rest, mxu = f - sum(vpu), []
    while rest > 0:
        n = 512 if rest > 512 else rest
        mxu.append(n)
        rest -= n
    mxu.sort(reverse=True)
    return tuple(mxu), vpu


def _kernel(x_hbm, wr_hbm, k_hbm, v_hbm, wq_hbm, wo_hbm, wg_hbm, wu_hbm, wd_hbm, o_ref,
            x_buf, wr_buf, wq_buf, k_buf, v_buf, wo_buf, wg_buf, wu_buf, wd_buf, sems):
    d = wq_buf.shape[0]
    hkv, w, _ = k_buf.shape
    sk = k_hbm.shape[2]
    f = wd_buf.shape[0]
    rep = HQ // hkv
    gw = rep * DH
    mxu_splits, vpu_splits = _down_splits(f)

    names, copies = [], {}

    def add(name, src, dst):
        copies[name] = pltpu.make_async_copy(src, dst, sems.at[len(names) % N_SEM])
        names.append(name)

    add("x", x_hbm, x_buf)
    add("wr", wr_hbm, wr_buf)
    rq = d // WQ_CHUNKS
    for c in range(WQ_CHUNKS):
        add(("wq", c), wq_hbm.at[pl.ds(c * rq, rq), :], wq_buf.at[pl.ds(c * rq, rq), :])
    for g in range(hkv):
        add(("k", g), k_hbm.at[0, g, pl.ds(sk - w, w), :], k_buf.at[g])
        add(("v", g), v_hbm.at[0, g, pl.ds(sk - w, w), :], v_buf.at[g])
        add(("wo", g), wo_hbm.at[pl.ds(g * gw, gw), :], wo_buf.at[pl.ds(g * gw, gw), :])
    add("wg", wg_hbm, wg_buf)
    add("wu", wu_hbm, wu_buf)
    wd_chunks, off = [], 0
    for i, n in enumerate(mxu_splits + vpu_splits):
        add(("wd", i), wd_hbm.at[pl.ds(off, n), :], wd_buf.at[pl.ds(off, n), :])
        wd_chunks.append((off, n))
        off += n

    n_started = [0]

    def start_upto(n):
        while n_started[0] < min(n, len(names)):
            copies[names[n_started[0]]].start()
            n_started[0] += 1

    def wait(name):
        copies[name].wait()
        start_upto(names.index(name) + 1 + N_SEM)

    start_upto(N_SEM)

    wait("x")
    x = x_buf[0].astype(jnp.float32)
    mean = jnp.mean(x, axis=-1, keepdims=True)
    xc = x - mean
    var = jnp.mean(xc * xc, axis=-1, keepdims=True)
    xn = (xc / jnp.sqrt(var + LN_EPS)).astype(jnp.bfloat16)
    xn8 = jnp.broadcast_to(xn, (8, d))
    xn_f = xn.astype(jnp.float32)
    wait("wr")
    wr = wr_buf[...].astype(jnp.float32).reshape(1, d)
    gate = jax.nn.sigmoid(jnp.sum(xn_f * wr, axis=-1, keepdims=True))

    q = None
    for c in range(WQ_CHUNKS):
        wait(("wq", c))
        part = _dot(xn8[:, c * rq:(c + 1) * rq], wq_buf[pl.ds(c * rq, rq), :])
        q = part if q is None else q + part

    row = jax.lax.broadcasted_iota(jnp.int32, (8, DH), 0) % rep
    blk_row = jax.lax.broadcasted_iota(jnp.int32, (8, gw), 0)
    blk_col = jax.lax.broadcasted_iota(jnp.int32, (8, gw), 1) // DH
    acc = jnp.zeros((8, d), jnp.float32)
    for g in range(hkv):
        qg = q[:, (rep * g) * DH:(rep * g + 1) * DH]
        for j in range(1, rep):
            qg = jnp.where(row == j, q[:, (rep * g + j) * DH:(rep * g + j + 1) * DH], qg)
        qg = qg.astype(jnp.bfloat16)
        wait(("k", g))
        s = _dot(qg, k_buf[g], _NT) * (DH ** -0.5)
        p = jnp.exp(s - jnp.max(s, axis=-1, keepdims=True))
        denom = jnp.sum(p, axis=-1, keepdims=True)
        wait(("v", g))
        o = _dot(p.astype(jnp.bfloat16), v_buf[g]) / denom
        o_blk = jnp.concatenate([o] * rep, axis=1)
        o_blk = jnp.where(blk_row == blk_col, o_blk, 0.0).astype(jnp.bfloat16)
        wait(("wo", g))
        acc = acc + _dot(o_blk, wo_buf[pl.ds(g * gw, gw), :])
    base = x + xn_f + jnp.sum(acc, axis=0, keepdims=True)

    wait("wg")
    gt = _dot(xn8, wg_buf[...])
    wait("wu")
    up = _dot(xn8, wu_buf[...])
    h = (gt * jax.nn.sigmoid(gt) * up).astype(jnp.bfloat16)

    vpu_off = sum(mxu_splits)
    h_cols = []
    for b in range(vpu_off, f, 128):
        h_row = jnp.broadcast_to(h[0:1, b:b + 128].astype(jnp.float32), (128, 128))
        h_cols.append(jnp.transpose(h_row))

    y = None
    for i, (off, n) in enumerate(wd_chunks[:len(mxu_splits)]):
        wait(("wd", i))
        part = _dot(h[:, off:off + n], wd_buf[pl.ds(off, n), :])
        y = part if y is None else y + part
    out = base + y[0:1] * gate

    y8 = None
    for i, (off, n) in list(enumerate(wd_chunks))[len(mxu_splits):]:
        wait(("wd", i))
        lo = off - vpu_off
        hb = h_cols[lo // 128][lo % 128:lo % 128 + n]
        prod = wd_buf[pl.ds(off, n), :].astype(jnp.float32) * jnp.concatenate([hb] * (d // 128), axis=1)
        part = jnp.sum(prod.reshape(n // 8, 8, d), axis=0)
        y8 = part if y8 is None else y8 + part
    if y8 is not None:
        out = out + jnp.sum(y8, axis=0, keepdims=True) * gate
    o_ref[0] = out.astype(o_ref.dtype)


@jax.jit
def pallas_parallel_sum__sliding_block_cached__moe_arch_mod__decode_kernel(
    A_x: jax.Array,
    A_k_cache: jax.Array,
    A_v_cache: jax.Array,
    A_wq: jax.Array,
    A_wo: jax.Array,
    B_x: jax.Array,
    B_w_r: jax.Array,
    B_w_gate: jax.Array,
    B_w_up: jax.Array,
    B_w_down: jax.Array,
):
    del B_x
    b, s, d = A_x.shape
    assert (b, s) == (1, 1), "decode kernel: one token"
    _, hkv, sk, dh = A_k_cache.shape
    assert dh == DH and HQ % hkv == 0 and 8 % (HQ // hkv) == 0
    w = min(4096, max(256, sk // 4))
    f = B_w_gate.shape[1]
    bf16 = jnp.bfloat16
    hbm = pl.BlockSpec(memory_space=pl.ANY)
    return pl.pallas_call(
        _kernel,
        out_shape=jax.ShapeDtypeStruct(A_x.shape, A_x.dtype),
        in_specs=[hbm] * 9,
        out_specs=pl.BlockSpec(memory_space=pltpu.VMEM),
        scratch_shapes=[
            pltpu.VMEM((1, 1, d), bf16),
            pltpu.VMEM((d,), bf16),
            pltpu.VMEM((d, HQ * DH), bf16),
            pltpu.VMEM((hkv, w, DH), bf16),
            pltpu.VMEM((hkv, w, DH), bf16),
            pltpu.VMEM((HQ * DH, d), bf16),
            pltpu.VMEM((d, f), bf16),
            pltpu.VMEM((d, f), bf16),
            pltpu.VMEM((f, d), bf16),
            pltpu.SemaphoreType.DMA((N_SEM,)),
        ],
        compiler_params=pltpu.CompilerParams(vmem_limit_bytes=64 * 1024 * 1024),
    )(A_x, B_w_r, A_k_cache, A_v_cache, A_wq, A_wo, B_w_gate, B_w_up, B_w_down)
```
